```python
import os as _os
_os.environ.setdefault("JAX_PLATFORMS", "cpu")
import jax
import jax.numpy as jnp

def _softmax(x, axis=-1):
    return jax.nn.softmax(x, axis=axis)
def _gelu(x):
    return jax.nn.gelu(x, approximate=True)
def _silu(x):
    return jax.nn.silu(x)
def _sigmoid(x):
    return jax.nn.sigmoid(x)
def _layernorm(x, axis=-1, eps=1e-5):
    m = jnp.mean(x, axis=axis, keepdims=True)
    v = jnp.var(x, axis=axis, keepdims=True)
    return (x - m) / jnp.sqrt(v + eps)
def _scatter_add(tgt, idx, src, axis=0):
    return tgt.at[idx].add(src)
def _segment_sum(src, seg, n):
    return jax.ops.segment_sum(src, seg, n)
class _Rng:
    def __init__(self, key):
        self._k = key
    def _next(self):
        self._k, sub = jax.random.split(self._k)
        return sub
    def normal(self, shape):
        return jax.random.normal(self._next(), shape, dtype=jnp.bfloat16)
    def randint(self, lo, hi, shape):
        return jax.random.randint(self._next(), shape, lo, hi, dtype=jnp.int32)
    def uniform(self, shape, lo=0.0, hi=1.0):
        return jax.random.uniform(self._next(), shape, jnp.bfloat16, lo, hi)
    def permutation(self, n):
        return jax.random.permutation(self._next(), n)


kernel_name = 'gated_mix__linear_kernel_hedgehog__glu_gated_bilinear__prompt'

def setup_inputs():
    _rng = _Rng(jax.random.key(int.from_bytes(__import__("os").urandom(4), "little")))
    _w = (lambda a: (lambda t: t.astype(jnp.bfloat16) if jnp.issubdtype(t.dtype, jnp.floating) else t)(jnp.asarray(a)))
    def _A_setup():
        B, S, D, H = 1, 2048, 512, 32
        Dh = D // H
        return {
            "x": _w((lambda *s: _rng.normal(s) * 0.05)(B, S, D)),
            "wqkv": _w((lambda *s: _rng.normal(s) * 0.8)(D, 3 * D)),
            "w_phi": _w((lambda *s: _rng.normal(s) * 0.8)(H, Dh, Dh) * (Dh ** -0.5)),
            "wo": _w((lambda *s: _rng.normal(s) * 0.05)(D, D)),
        }
    _A_in = _A_setup()

    def _B_setup():
        B, S, D, F = 1, 2048, 512, 1792
        return {
            "x": _w((lambda *s: _rng.normal(s) * 0.05)(B, S, D)),
            "w_gate": _w((lambda *s: _rng.normal(s) * 1.6)(D, F) * (D ** -0.5)),
            "w_up": _w((lambda *s: _rng.normal(s) * 1.6)(D, F) * (D ** -0.5)),
            "w_down": _w((lambda *s: _rng.normal(s) * 1.6)(F, D) * (F ** -0.5)),
        }
    _B_in = _B_setup()

    return {
        "A_x": _A_in["x"],
        "A_wqkv": _A_in["wqkv"],
        "A_w_phi": _A_in["w_phi"],
        "A_wo": _A_in["wo"],
        "B_x": _B_in["x"],
        "B_w_gate": _B_in["w_gate"],
        "B_w_up": _B_in["w_up"],
        "B_w_down": _B_in["w_down"],
        "gate_w": _w((lambda *s: _rng.normal(s) * 0.05)(512) * 16.0),
    }

def reference(A_x, A_wqkv, A_w_phi, A_wo, B_x, B_w_gate, B_w_up, B_w_down, gate_w):
    def _A_ref(x, wqkv, w_phi, wo):
        B, S, D = x.shape
        H = 32; Dh = D // H
        qkv = (lambda x, *d: x.transpose(*d))((x @ wqkv).reshape(B, S, 3, H, Dh), 2, 0, 3, 1, 4)
        q, k, v = qkv[0], qkv[1], qkv[2]
        pq = jnp.einsum("bhsd,hdf->bhsf", q, w_phi)
        pk = jnp.einsum("bhsd,hdf->bhsf", k, w_phi)
        phi_q = jnp.concatenate([_softmax(pq, axis=-1), _softmax(-pq, axis=-1)], axis=-1)
        phi_k = jnp.concatenate([_softmax(pk, axis=-1), _softmax(-pk, axis=-1)], axis=-1)
        kv = jnp.einsum("bhsf,bhsd->bhfd", phi_k, v)
        z  = jnp.einsum("bhsf->bhf", phi_k)
        num = jnp.einsum("bhqf,bhfd->bhqd", phi_q, kv)
        den = jnp.einsum("bhqf,bhf->bhq", phi_q, z)[..., None] + 1e-6
        o = num / den
        return (lambda x, *d: x.transpose(*d))(o, 0, 2, 1, 3).reshape(B, S, D) @ wo

    def _B_ref(x, w_gate, w_up, w_down):
        g = jnp.einsum("bsd,df->bsf", x, w_gate)
        u = jnp.einsum("bsd,df->bsf", x, w_up)
        h = g * u
        return jnp.einsum("bsf,fd->bsd", h, w_down)

    x = A_x
    g = _sigmoid((x * gate_w).sum(-1, keepdims=True))
    a = _A_ref(x, A_wqkv, A_w_phi, A_wo)
    b = _B_ref(x, B_w_gate, B_w_up, B_w_down)
    return g * a + (1 - g) * b
```

```python
import jax
import jax.numpy as jnp
import jax.experimental.pallas as pl
import jax.experimental.pallas.tpu as pltpu

_H = 32
_LOG2E = 1.4426950408889634
_TA = 512
_TB = 512
_TF = 1792
_BF = jnp.bfloat16
_F32 = jnp.float32


def _nn(a, b):
    return jax.lax.dot_general(a, b, (((1,), (0,)), ((), ())), preferred_element_type=_F32)


def _nt(a, b):
    return jax.lax.dot_general(a, b, (((1,), (1,)), ((), ())), preferred_element_type=_F32)


def _tn(a, b):
    return jax.lax.dot_general(a, b, (((0,), (0,)), ((), ())), preferred_element_type=_F32)


def _iota(shape, d):
    return jax.lax.broadcasted_iota(jnp.int32, shape, d)


def _kernel(x_hbm, wqkv_hbm, wphi_ref, wo_hbm, wg_hbm, wu_hbm, wd_hbm, gw_ref, out_hbm,
            x_v, wqkv_v, wo_v, wg_v, wu_v, wd_v, out_v,
            wqkt_v, wvp_v, wop_v, phiq_v, kv_v, z_v, lhs_v,
            sem_x, sem_w, sem_o):
    S, D = x_v.shape
    F = wg_v.shape[1]
    G = D // 128
    nA = S // _TA
    nB = S // _TB

    def x_copy(i):
        return pltpu.make_async_copy(x_hbm.at[pl.ds(i * _TA, _TA)], x_v.at[pl.ds(i * _TA, _TA)], sem_x.at[i])

    def o_copy(i):
        return pltpu.make_async_copy(out_v.at[pl.ds(i * _TB, _TB)], out_hbm.at[pl.ds(i * _TB, _TB)], sem_o.at[i])

    c_qkv = pltpu.make_async_copy(wqkv_hbm, wqkv_v, sem_w.at[0])
    c_wg = pltpu.make_async_copy(wg_hbm, wg_v, sem_w.at[1])
    c_wu = pltpu.make_async_copy(wu_hbm, wu_v, sem_w.at[2])
    c_wd = pltpu.make_async_copy(wd_hbm, wd_v, sem_w.at[3])
    c_wo = pltpu.make_async_copy(wo_hbm, wo_v, sem_w.at[4])

    c_qkv.start()
    x_copy(0).start()
    c_qkv.wait()
    for i in range(1, nA):
        x_copy(i).start()
    c_wo.start()
    c_wg.start()
    c_wu.start()
    c_wd.start()

    r = _iota((128, 128), 0)
    c = _iota((128, 128), 1)
    et = (_iota((128, 16), 0) // 8 == _iota((128, 16), 1)).astype(_BF)
    head_sel = (c // 16) == (r % 8)
    perm = ((c % 8) * 16 + c // 8 == r).astype(_BF)
    permt = ((r % 8) * 16 + r // 8 == c).astype(_BF)
    for j in range(G):
        wp = wphi_ref[pl.ds(j * 128, 128), :]
        bt = jnp.where(head_sel, _nt(et, wp), 0.0).astype(_BF)
        for t in range(2):
            w = wqkv_v[:, pl.ds(t * D + j * 128, 128)]
            wqkt_v[pl.ds(t * D + j * 128, 128), :] = (_nt(bt, w) * _LOG2E).astype(_BF)
        wvp_v[:, pl.ds(j * 128, 128)] = _nn(wqkv_v[:, pl.ds(2 * D + j * 128, 128)], perm).astype(_BF)

    kv_v[...] = jnp.zeros(kv_v.shape, _F32)
    z_v[...] = jnp.zeros(z_v.shape, _F32)

    def dual_softmax(p):
        p3 = p.reshape(16, 8, _TA)
        mx = jnp.max(p3, axis=0, keepdims=True)
        mn = jnp.min(p3, axis=0, keepdims=True)
        ep = jnp.exp2(p3 - mx)
        en = jnp.exp2(mn - p3)
        ep = ep * (1.0 / jnp.sum(ep, axis=0, keepdims=True))
        en = en * (1.0 / jnp.sum(en, axis=0, keepdims=True))
        return jnp.concatenate([ep.reshape(128, _TA), en.reshape(128, _TA)], axis=0)

    def phase_a(i, _):
        x_copy(i).wait()
        rows = pl.ds(pl.multiple_of(i * _TA, _TA), _TA)
        xb = x_v[rows, :]
        pt = _nt(wqkt_v[...], xb)
        v = _nn(xb, wvp_v[...]).astype(_BF)
        for j in range(G):
            ph = dual_softmax(pt[D + j * 128:D + (j + 1) * 128])
            zs = ph[:, 0:128]
            for l in range(1, _TA // 128):
                zs = zs + ph[:, l * 128:(l + 1) * 128]
            z_v[j] += zs
            kv_v[j] += _nn(ph.astype(_BF), v[:, j * 128:(j + 1) * 128])
        for j in range(G):
            phiq_v[j, :, rows] = dual_softmax(pt[j * 128:(j + 1) * 128]).astype(_BF)
        return _

    jax.lax.fori_loop(0, nA, phase_a, 0)

    c_wo.wait()
    r2 = _iota((128, 256), 0)
    c2 = _iota((128, 256), 1)
    same = (r2 % 8) == (c2 % 8)
    r3 = _iota((16, 256), 0)
    c3 = _iota((16, 256), 1)
    for j in range(G):
        wop_v[pl.ds(j * 128, 128), :] = _nn(permt, wo_v[pl.ds(j * 128, 128), :]).astype(_BF)
        lhs_v[j, pl.ds(0, 128), :] = jnp.where(same, kv_v[j].T, 0.0).astype(_BF)
        zrow = jnp.sum(z_v[j].T, axis=0, keepdims=True)
        lhs_v[j, pl.ds(128, 16), :] = jnp.where(r3 == (c3 % 8), zrow, 0.0).astype(_BF)
    c_wg.wait()
    c_wu.wait()
    c_wd.wait()

    gw = gw_ref[...].astype(_F32)

    def phase_b(i, _):
        rows = pl.ds(pl.multiple_of(i * _TB, _TB), _TB)
        xb = x_v[rows, :]
        ots = []
        for j in range(G):
            nd = _nn(lhs_v[j], phiq_v[j, :, rows])
            inv = 1.0 / (nd[128:136] + 1e-6)
            ots.append((nd[0:128].reshape(16, 8, _TB) * inv[None]).reshape(128, _TB))
        ot = jnp.concatenate(ots, axis=0)
        a = _nn(ot.T.astype(_BF), wop_v[...])
        b = None
        for f in range(F // _TF):
            cols = pl.ds(f * _TF, _TF)
            h = (_nn(xb, wg_v[:, cols]) * _nn(xb, wu_v[:, cols])).astype(_BF)
            d = _nn(h, wd_v[cols, :])
            b = d if b is None else b + d
        g = jax.nn.sigmoid(jnp.sum(xb.astype(_F32) * gw, axis=-1, keepdims=True))
        out_v[rows, :] = (g * a + (1.0 - g) * b).astype(out_v.dtype)
        o_copy(i).start()
        return _

    jax.lax.fori_loop(0, nB, phase_b, 0)
    for i in range(nB):
        o_copy(i).wait()


@jax.jit
def pallas_gated_mix__linear_kernel_hedgehog__glu_gated_bilinear__prompt_kernel(
    A_x: jax.Array,
    A_wqkv: jax.Array,
    A_w_phi: jax.Array,
    A_wo: jax.Array,
    B_x: jax.Array,
    B_w_gate: jax.Array,
    B_w_up: jax.Array,
    B_w_down: jax.Array,
    gate_w: jax.Array,
):
    del B_x
    B, S, D = A_x.shape
    F = B_w_gate.shape[1]
    G = D // 128
    assert B == 1 and D == _H * 16
    hbm = pl.BlockSpec(memory_space=pl.ANY)
    vmem = pl.BlockSpec(memory_space=pltpu.VMEM)
    out = pl.pallas_call(
        _kernel,
        out_shape=jax.ShapeDtypeStruct((S, D), A_x.dtype),
        in_specs=[hbm, hbm, vmem, hbm, hbm, hbm, hbm, vmem],
        out_specs=hbm,
        scratch_shapes=[
            pltpu.VMEM((S, D), _BF), pltpu.VMEM((D, 3 * D), _BF), pltpu.VMEM((D, D), _BF),
            pltpu.VMEM((D, F), _BF), pltpu.VMEM((D, F), _BF), pltpu.VMEM((F, D), _BF),
            pltpu.VMEM((S, D), A_x.dtype),
            pltpu.VMEM((2 * D, D), _BF), pltpu.VMEM((D, D), _BF), pltpu.VMEM((D, D), _BF),
            pltpu.VMEM((G, 256, S), _BF), pltpu.VMEM((G, 256, 128), _F32),
            pltpu.VMEM((G, 256, 128), _F32), pltpu.VMEM((G, 144, 256), _BF),
            pltpu.SemaphoreType.DMA((S // _TA,)), pltpu.SemaphoreType.DMA((5,)),
            pltpu.SemaphoreType.DMA((S // _TB,)),
        ],
        compiler_params=pltpu.CompilerParams(vmem_limit_bytes=100 * 1024 * 1024),
    )(A_x.reshape(S, D), A_wqkv, A_w_phi.reshape(D, 16), A_wo, B_w_gate, B_w_up, B_w_down,
      gate_w.reshape(1, D))
    return out.reshape(B, S, D)
```

```python
import jax
import jax.numpy as jnp
import jax.experimental.pallas as pl
import jax.experimental.pallas.tpu as pltpu

_H = 32
_LOG2E = 1.4426950408889634
_TA = 512
_TB = 512
_N = 2
_P = {2: 7, 4: 49}[_N]
_CW = 896
_BF = jnp.bfloat16
_F32 = jnp.float32


def _nn(a, b):
    return jax.lax.dot_general(a, b, (((1,), (0,)), ((), ())), preferred_element_type=_F32)


def _nt(a, b):
    return jax.lax.dot_general(a, b, (((1,), (1,)), ((), ())), preferred_element_type=_F32)


def _iota(shape, d):
    return jax.lax.broadcasted_iota(jnp.int32, shape, d)


def _rhs7(b11, b12, b21, b22):
    return [b11 + b22, b11, b12 - b22, b21 - b11, b22, b11 + b12, b21 + b22]


def _lhs7(a11, a12, a21, a22):
    return [a11 + a22, a21 + a22, a11, a22, a11 + a12, a21 - a11, a12 - a22]


def _expand(f7, m):
    n = len(m)
    if n == 1:
        return [m[0][0]]
    h = n // 2
    parts = [[f7(m[i][j], m[i][j + h], m[i + h][j], m[i + h][j + h]) for j in range(h)] for i in range(h)]
    out = []
    for k in range(7):
        out += _expand(f7, [[parts[i][j][k] for j in range(h)] for i in range(h)])
    return out


def _combine(ms):
    if len(ms) == 1:
        return [[ms[0]]]
    n = len(ms) // 7
    sub = [_combine(ms[k * n:(k + 1) * n]) for k in range(7)]
    h = len(sub[0])
    out = [[None] * (2 * h) for _ in range(2 * h)]
    for i in range(h):
        for j in range(h):
            (out[i][j], out[i][j + h], out[i + h][j], out[i + h][j + h]) = _strassen_out(
                [sub[k][i][j] for k in range(7)])
    return out


def _strassen_out(m):
    return m[0] + m[3] - m[4] + m[6], m[2] + m[4], m[1] + m[3], m[0] - m[1] + m[2] + m[5]


def _kernel(x_hbm, wqkv_hbm, wphi_hbm, wo_hbm, wg_hbm, wu_hbm, wd_hbm, gw_hbm, out_hbm,
            x_v, wqkv_v, wo_v, wg_v, wu_v, wd_v, out_v, wphi_v, gw_v,
            wqkt_v, phiq_v, kv_v, z_v, lhs_v, sgu_v, sd_v,
            sem_x, sem_w, sem_o):
    S, D = x_v.shape
    F = wg_v.shape[1]
    G = D // 128
    nA = S // _TA
    nB = S // _TB
    hD, hF, hB = D // 2, F // 2, _TB // 2

    def x_copy(i):
        return pltpu.make_async_copy(x_hbm.at[pl.ds(i * _TA, _TA)], x_v.at[pl.ds(i * _TA, _TA)], sem_x.at[i])

    def o_copy(i):
        return pltpu.make_async_copy(out_v.at[pl.ds(i * hB, hB)], out_hbm.at[pl.ds(i * hB, hB)], sem_o.at[i])

    c_qk = pltpu.make_async_copy(wqkv_hbm.at[:, pl.ds(0, 2 * D)], wqkv_v.at[:, pl.ds(0, 2 * D)], sem_w.at[0])
    c_v = pltpu.make_async_copy(wqkv_hbm.at[:, pl.ds(2 * D, D)], wqkv_v.at[:, pl.ds(2 * D, D)], sem_w.at[7])
    c_wg = pltpu.make_async_copy(wg_hbm, wg_v, sem_w.at[1])
    c_wu = pltpu.make_async_copy(wu_hbm, wu_v, sem_w.at[2])
    c_wd = pltpu.make_async_copy(wd_hbm, wd_v, sem_w.at[3])
    c_wo = pltpu.make_async_copy(wo_hbm, wo_v, sem_w.at[4])
    c_phi = pltpu.make_async_copy(wphi_hbm, wphi_v, sem_w.at[5])
    c_gw = pltpu.make_async_copy(gw_hbm, gw_v, sem_w.at[6])

    c_phi.start()
    c_qk.start()
    x_copy(0).start()
    c_v.start()
    c_phi.wait()

    sel = (_iota((_H, D), 1) // 16 == _iota((_H, D), 0)).astype(_BF)
    t = _nn(wphi_v[...], sel)
    t = jnp.where(_iota((256, D), 0) // 16 == _iota((256, D), 1) % 16, t, 0.0).astype(_BF)
    rep = ((_iota((128, 256), 0) % 64) // 4 == _iota((128, 256), 1) % 16).astype(_BF)
    bt = jnp.where((_iota((128, D), 1) // 16) % 8 == (_iota((128, D), 0) // 64) * 4 + _iota((128, D), 0) % 4, _nn(rep, t), 0.0).astype(_BF)
    kv_v[...] = jnp.zeros(kv_v.shape, _F32)
    z_v[...] = jnp.zeros(z_v.shape, _F32)

    c_qk.wait()
    for i in range(1, nA):
        x_copy(i).start()
    c_wg.start()
    c_wu.start()
    c_wd.start()
    c_wo.start()
    c_gw.start()
    for j in range(G):
        for s in range(2):
            w = wqkv_v[:, pl.ds(s * D + j * 128, 128)]
            wqkt_v[pl.ds(s * D + j * 128, 128), :] = (
                _nt(bt[:, j * 128:(j + 1) * 128], w) * _LOG2E).astype(_BF)
    c_v.wait()

    def dual_softmax(p):
        p3 = p.reshape(8, 8, _TA)

        def red(full, pair, y):
            y = full(y, axis=0)
            return pair(y, pltpu.roll(y, 4, 0))[None]
        ep = jnp.exp2(p3 - red(jnp.max, jnp.maximum, p3))
        en = jnp.exp2(red(jnp.min, jnp.minimum, p3) - p3)
        ep = ep * (1.0 / red(jnp.sum, jnp.add, ep))
        en = en * (1.0 / red(jnp.sum, jnp.add, en))
        return jnp.concatenate([ep.reshape(64, _TA), en.reshape(64, _TA)], axis=0)

    def phase_a(i, extra):
        rows = pl.ds(pl.multiple_of(i * _TA, _TA), _TA)
        xb = x_v[rows, :]
        pt = _nt(wqkt_v[...], xb)
        v = _nn(xb, wqkv_v[:, pl.ds(2 * D, D)]).T.astype(_BF)
        for j in range(2 * G):
            ph = dual_softmax(pt[D + j * 64:D + (j + 1) * 64])
            zs = ph[:, 0:128]
            for l in range(1, _TA // 128):
                zs = zs + ph[:, l * 128:(l + 1) * 128]
            z_v[j] += zs
            kv_v[j] += _nt(v[j * 64:(j + 1) * 64], ph.astype(_BF))
        for j in range(2 * G):
            phiq_v[j, :, rows] = dual_softmax(pt[j * 64:(j + 1) * 64]).astype(_BF)
        extra()

    def a_body(i, c):
        x_copy(i).wait()
        phase_a(i, lambda: None)
        return c

    jax.lax.fori_loop(0, nA // 2, a_body, 0)

    c_wg.wait()
    c_wu.wait()
    c_wd.wait()
    kq = D // _N
    fq = 2 * F // _N

    def prep(t, s):
        n = kq // (nA - nA // 2)
        w7 = fq // 7
        for r in range(0, n, 16):
            r0 = pl.multiple_of(t * n + r, 16)
            for c in range(s * w7, (s + 1) * w7, 128):
                m = [[(wg_v if b < _N // 2 else wu_v)[pl.ds(a * kq + r0, 16),
                                                     pl.ds((b % (_N // 2)) * fq + c, 128)].astype(_F32)
                      for b in range(_N)] for a in range(_N)]
                for k, w in enumerate(_expand(_rhs7, m)):
                    sgu_v[k, pl.ds(r0, 16), pl.ds(c, 128)] = w.astype(_BF)

    def prep_d(t):
        n = hF // (nA - nA // 2)
        for r in range(0, n, 16):
            r0 = pl.multiple_of(t * n + r, 16)
            m = [[wd_v[pl.ds(a * hF + r0, 16), pl.ds(b * hD, hD)].astype(_F32)
                  for b in range(2)] for a in range(2)]
            for k, w in enumerate(_expand(_rhs7, m)):
                sd_v[k, pl.ds(r0, 16), :] = w.astype(_BF)

    def a_body2(i, c):
        x_copy(i).wait()
        t = i - nA // 2

        def extra():
            prep_d(t)
            for s in range(7):
                prep(t, s)
        phase_a(i, extra)
        return c

    jax.lax.fori_loop(nA // 2, nA, a_body2, 0)

    same = _iota((64, 128), 0) // 16 == _iota((64, 128), 1) % 4
    zsel = _iota((16, 128), 0) == _iota((16, 128), 1) % 4
    for j in range(2 * G):
        lhs_v[j, pl.ds(0, 64), :] = jnp.where(same, kv_v[j], 0.0).astype(_BF)
        zrow = jnp.sum(z_v[j].T, axis=0, keepdims=True)
        lhs_v[j, pl.ds(64, 16), :] = jnp.where(zsel, zrow, 0.0).astype(_BF)
    c_wo.wait()
    c_gw.wait()

    gw = gw_v[...].astype(_F32).reshape(1, D)

    def phase_b(i, c):
        rows = pl.ds(pl.multiple_of(i * _TB, _TB), _TB)
        xf = x_v[rows, :].astype(_F32)
        ots = []
        for j in range(2 * G):
            nd = _nn(lhs_v[j], phiq_v[j, :, rows])
            inv = 1.0 / (nd[64:72] + 1e-6)
            for h in range(4):
                ots.append(nd[h * 16:(h + 1) * 16] * inv[h:h + 1])
        ot = jnp.concatenate(ots, axis=0)
        a = _nn(ot.T.astype(_BF), wo_v[...])
        rq = _TB // _N
        xs = [w.astype(_BF) for w in _expand(_lhs7, [
            [xf[a * rq:(a + 1) * rq, b * kq:(b + 1) * kq] for b in range(_N)] for a in range(_N)])]
        parts = {}
        for c in range(0, fq, _CW):
            o = _combine([_nn(xs[k], sgu_v[k, :, pl.ds(c, _CW)]) for k in range(_P)])
            for b in range(_N // 2):
                parts[b * fq + c] = jnp.concatenate(
                    [o[a][b] * o[a][b + _N // 2] for a in range(_N)], axis=0)
        hl = [[] for _ in range(7)]
        for c in range(0, hF, _CW):
            h1, h2 = parts[c], parts[hF + c]
            for k, w in enumerate(_lhs7(h1[:hB], h2[:hB], h1[hB:], h2[hB:])):
                hl[k].append(w.astype(_BF))
        hl = [jnp.concatenate(w, axis=1) for w in hl]
        b11, b12, b21, b22 = _strassen_out([_nn(hl[k], sd_v[k]) for k in range(7)])
        b = jnp.concatenate([jnp.concatenate([b11, b12], axis=1),
                             jnp.concatenate([b21, b22], axis=1)], axis=0)
        g = jax.nn.sigmoid(jnp.sum(xf * gw, axis=-1, keepdims=True))
        out_v[rows, :] = (g * a + (1.0 - g) * b).astype(out_v.dtype)
        o_copy(2 * i).start()
        o_copy(2 * i + 1).start()
        return c

    jax.lax.fori_loop(0, nB, phase_b, 0)
    for i in range(2 * nB):
        o_copy(i).wait()


@jax.jit
def pallas_gated_mix__linear_kernel_hedgehog__glu_gated_bilinear__prompt_kernel(
    A_x: jax.Array,
    A_wqkv: jax.Array,
    A_w_phi: jax.Array,
    A_wo: jax.Array,
    B_x: jax.Array,
    B_w_gate: jax.Array,
    B_w_up: jax.Array,
    B_w_down: jax.Array,
    gate_w: jax.Array,
):
    del B_x
    B, S, D = A_x.shape
    F = B_w_gate.shape[1]
    G = D // 128
    assert B == 1 and D == _H * 16
    hbm = pl.BlockSpec(memory_space=pl.ANY)
    out = pl.pallas_call(
        _kernel,
        out_shape=jax.ShapeDtypeStruct((S, D), A_x.dtype),
        in_specs=[hbm] * 8,
        out_specs=hbm,
        scratch_shapes=[
            pltpu.VMEM((S, D), _BF), pltpu.VMEM((D, 3 * D), _BF), pltpu.VMEM((D, D), _BF),
            pltpu.VMEM((D, F), _BF), pltpu.VMEM((D, F), _BF), pltpu.VMEM((F, D), _BF),
            pltpu.VMEM((S, D), A_x.dtype), pltpu.VMEM((256, _H), _BF), pltpu.VMEM((D,), _BF),
            pltpu.VMEM((2 * D, D), _BF),
            pltpu.VMEM((2 * G, 128, S), _BF), pltpu.VMEM((2 * G, 64, 128), _F32),
            pltpu.VMEM((2 * G, 128, 128), _F32), pltpu.VMEM((2 * G, 80, 128), _BF),
            pltpu.VMEM((_P, D // _N, 2 * F // _N), _BF), pltpu.VMEM((7, F // 2, D // 2), _BF),
            pltpu.SemaphoreType.DMA((S // _TA,)), pltpu.SemaphoreType.DMA((8,)),
            pltpu.SemaphoreType.DMA((2 * S // _TB,)),
        ],
        compiler_params=pltpu.CompilerParams(vmem_limit_bytes=110 * 1024 * 1024),
    )(A_x.reshape(S, D), A_wqkv, A_w_phi.transpose(1, 2, 0).reshape(256, _H), A_wo,
      B_w_gate, B_w_up, B_w_down, gate_w)
    return out.reshape(B, S, D)
```
